```python
import os as _os
_os.environ.setdefault("JAX_PLATFORMS", "cpu")
import jax
import jax.numpy as jnp

def _softmax(x, axis=-1):
    return jax.nn.softmax(x, axis=axis)
def _gelu(x):
    return jax.nn.gelu(x, approximate=True)
def _silu(x):
    return jax.nn.silu(x)
def _sigmoid(x):
    return jax.nn.sigmoid(x)
def _layernorm(x, axis=-1, eps=1e-5):
    m = jnp.mean(x, axis=axis, keepdims=True)
    v = jnp.var(x, axis=axis, keepdims=True)
    return (x - m) / jnp.sqrt(v + eps)
def _scatter_add(tgt, idx, src, axis=0):
    return tgt.at[idx].add(src)
def _segment_sum(src, seg, n):
    return jax.ops.segment_sum(src, seg, n)
class _Rng:
    def __init__(self, key):
        self._k = key
    def _next(self):
        self._k, sub = jax.random.split(self._k)
        return sub
    def normal(self, shape):
        return jax.random.normal(self._next(), shape, dtype=jnp.bfloat16)
    def randint(self, lo, hi, shape):
        return jax.random.randint(self._next(), shape, lo, hi, dtype=jnp.int32)
    def uniform(self, shape, lo=0.0, hi=1.0):
        return jax.random.uniform(self._next(), shape, jnp.bfloat16, lo, hi)
    def permutation(self, n):
        return jax.random.permutation(self._next(), n)


kernel_name = 'interleave_layers__sliding_local_dilated__moe_arch_mod__prompt'

def setup_inputs():
    _rng = _Rng(jax.random.key(int.from_bytes(__import__("os").urandom(4), "little")))
    _w = (lambda a: (lambda t: t.astype(jnp.bfloat16) if jnp.issubdtype(t.dtype, jnp.floating) else t)(jnp.asarray(a)))
    def _A_setup():
        B, S, D = 1, 2048, 512
        return {
            "x": _w((lambda *s: _rng.normal(s) * 0.05)(B, S, D)),
            "wqkv": _w((lambda *s: _rng.normal(s) * 0.05)(D, 3 * D)),
            "wo": _w((lambda *s: _rng.normal(s) * 0.05)(D, D)),
        }
    _A_in = _A_setup()

    def _B_setup():
        B, S, D, F, C = 1, 2048, 512, 1376, 2
        return {
            "x": _w((lambda *s: _rng.normal(s) * 0.05)(B, S, D)),
            "w_r": _w((lambda *s: _rng.normal(s) * 0.05)(D)),
            "w_gate": _w((lambda *s: _rng.normal(s) * 0.05)(D, F)),
            "w_up": _w((lambda *s: _rng.normal(s) * 0.05)(D, F)),
            "w_down": _w((lambda *s: _rng.normal(s) * 0.05)(F, D)),
        }
    _B_in = _B_setup()

    return {
        "A_x": _A_in["x"],
        "A_wqkv": _A_in["wqkv"],
        "A_wo": _A_in["wo"],
        "B_x": _B_in["x"],
        "B_w_r": _B_in["w_r"],
        "B_w_gate": _B_in["w_gate"],
        "B_w_up": _B_in["w_up"],
        "B_w_down": _B_in["w_down"],
    }

def reference(A_x, A_wqkv, A_wo, B_x, B_w_r, B_w_gate, B_w_up, B_w_down):
    def _A_ref(x, wqkv, wo):
        B, S, D = x.shape
        H = 32; Dh = D // H
        W, dil = 8, 2
        qkv = (lambda x, *d: x.transpose(*d))((x @ wqkv).reshape(B, S, 3, H, Dh), 2, 0, 3, 1, 4)
        q, k, v = qkv[0], qkv[1], qkv[2]
        scale = Dh ** -0.5
        pos = jnp.arange(S)
        off = jnp.arange(W) * dil
        idx = pos[:, None] - off[None, :]
        mask = idx >= 0
        idx_c = jnp.where(mask, idx, 0).reshape(-1)
        kg = k[:, :, idx_c, :].reshape(B, H, S, W, Dh)
        vg = v[:, :, idx_c, :].reshape(B, H, S, W, Dh)
        logits = jnp.einsum("bhsd,bhswd->bhsw", q, kg) * scale
        logits = jnp.where(mask[None, None, :, :], logits, -1e9)
        attn = _softmax(logits, axis=-1)
        o = jnp.einsum("bhsw,bhswd->bhsd", attn, vg)
        return (lambda x, *d: x.transpose(*d))(o, 0, 2, 1, 3).reshape(B, S, D) @ wo

    def _B_ref(x, w_r, w_gate, w_up, w_down):
        B, S, D = x.shape
        C = 2
        r = x @ w_r
        idx = jnp.argsort(-r, axis=-1)[:, :C]
        idx_e = jnp.repeat(idx.reshape(B, C, 1), D, axis=2)
        x_sel = jnp.take_along_axis(x, idx_e, axis=1)
        g = _silu(x_sel @ w_gate)
        u = x_sel @ w_up
        y = (g * u) @ w_down
        r_sel = _sigmoid(jnp.take_along_axis(r, idx, axis=1))
        y = y * r_sel.reshape(B, C, 1)
        b_off = (jnp.arange(B) * S).reshape(B, 1)
        flat_idx = (idx + b_off).reshape(B * C)
        zero = (x * 0.0).reshape(B * S, D)
        upd = _scatter_add(zero, flat_idx, y.reshape(B * C, D), axis=0)
        return x + upd.reshape(B, S, D)

    x = A_x
    x = x + _A_ref(_layernorm(x, axis=-1), A_wqkv, A_wo)
    x = x + _B_ref(_layernorm(x, axis=-1), B_w_r, B_w_gate, B_w_up, B_w_down)
    x = x + _A_ref(_layernorm(x, axis=-1), A_wqkv, A_wo)
    x = x + _B_ref(_layernorm(x, axis=-1), B_w_r, B_w_gate, B_w_up, B_w_down)
    return x
```

```python
import functools
import numpy as np
import jax
import jax.numpy as jnp
from jax import lax
import jax.experimental.pallas as pl
import jax.experimental.pallas.tpu as pltpu

S, D, F = 2048, 512, 1376
NW, DIL = 8, 2
PAD = 16
RC = 16
LOG2E = 1.4426950408889634
QSCALE = 0.25 * LOG2E
NEG = -1e9 * LOG2E
EPS = 1e-5
f32, bf16, u32 = jnp.float32, jnp.bfloat16, jnp.uint32


def _lane_iota(rows):
    return lax.broadcasted_iota(jnp.int32, (rows, 128), 1)


def _sum4(a):
    return (a[0] + a[1]) + (a[2] + a[3])


def _rowsum(x):
    return jnp.broadcast_to(jnp.sum(x, axis=1, keepdims=True), x.shape)


def _pack(x):
    return pltpu.bitcast(x.astype(bf16), u32)


def _ln_parts(xs):
    m = _rowsum(_sum4(xs)) * (1.0 / D)
    xc = [x - m for x in xs]
    v = _rowsum(_sum4([c * c for c in xc])) * (1.0 / D)
    return xc, lax.rsqrt(v + EPS)


def _kernel(x_hbm, wqkv_hbm, wo_hbm, wr_hbm, wg_hbm, wu_hbm, wd_hbm, out_hbm,
            xb, wraw, wp, woraw, wof, wop, wr_v, wg_v, wu_v, wd_v,
            hb0, hb1, qb0, qb1, kb0, kb1, vb0, vb1, ob0, ob1, xo0, xo1, x1b, rb, sa, sb, sc_, sma, smb, fix,
            sem_x, sem_w, sem_o, *, M, hops, lag, only_body, stage_ln):
    NB = S // M
    NCH = M // RC
    hb, qb, kb, vb, ob, xo = (hb0, hb1), (qb0, qb1), (kb0, kb1), (vb0, vb1), (ob0, ob1), (xo0, xo1)

    def rows(b, off=0, n=M):
        if isinstance(b, int):
            return pl.ds(b * M + off, n)
        return pl.ds(pl.multiple_of(b * M + off, RC), n)

    def x_copy(b):
        return pltpu.make_async_copy(x_hbm.at[0, rows(b)], xb.at[rows(b)], sem_x.at[b])

    def o_copy(b, p):
        return pltpu.make_async_copy(xo[p], out_hbm.at[0, rows(b)], sem_o.at[p])

    def r_copy(b, p):
        return pltpu.make_async_copy(xo[p], xb.at[rows(b)], sem_o.at[p])

    def w_copy(j):
        return pltpu.make_async_copy(wqkv_hbm.at[:, pl.ds(j * D, D)], wraw.at[j], sem_w.at[j])

    wo_copy = pltpu.make_async_copy(wo_hbm, woraw, sem_w.at[3])
    wr_copy = pltpu.make_async_copy(wr_hbm, wr_v, sem_w.at[4])
    wg_copy = pltpu.make_async_copy(wg_hbm, wg_v, sem_w.at[5])
    wu_copy = pltpu.make_async_copy(wu_hbm, wu_v, sem_w.at[6])
    wd_copy = pltpu.make_async_copy(wd_hbm, wd_v, sem_w.at[7])

    def permute_w(j):
        src = wraw.at[j].bitcast(u32)
        R = 32
        lane = _lane_iota(R)
        c0 = ((lane >> 2) & 1) == 1
        c1 = ((lane >> 3) & 1) == 1
        for r in range(0, D // 2, R):
            a = [src[pl.ds(r, R), pl.ds(i * 128, 128)] for i in range(4)]
            b = [jnp.where(c0, a[i ^ 1], a[i]) for i in range(4)]
            m = [jnp.where(c1, b[i ^ 2], b[i]) for i in range(4)]
            for t in range(4):
                idx = (lane & 7) * 16 + (((lane >> 3) & 3) ^ t) * 4 + (lane >> 5)
                wp[j * 4 + t, pl.ds(r, R), :] = jnp.take_along_axis(m[t], idx, axis=1)

    def permute_wo():
        for n in range(4):
            for r in range(0, D, 64):
                wof[n, pl.ds(r, 64), :] = woraw[pl.ds(r, 64), pl.ds(n * 128, 128)].astype(f32)
        for n in range(4):
            for t in range(4):
                for g in range(4):
                    parts = [wof[n, pl.ds(i * 128 + (i ^ t) * 4 + g, 8, stride=16), :] for i in range(4)]
                    wop[n, pl.ds(t * 64 + g * 16, 16), :] = _pack(jnp.concatenate(parts, axis=0))

    def ldx(b, c):
        return [xb[rows(b, c * RC, RC), pl.ds(i * 128, 128)].astype(f32) for i in range(4)]

    def ln_a(b, p, c):
        xc, inv = _ln_parts(ldx(b, c))
        for i in range(4):
            hb[p][pl.ds(c * 8, 8), pl.ds(i * 128, 128)] = _pack(xc[i] * inv)

    def ln_a1(b, p, c):
        sma[pl.ds(c * RC, RC), :] = _rowsum(_sum4(ldx(b, c))) * (1.0 / D)

    def ln_a2(b, p, c):
        m = sma[pl.ds(c * RC, RC), :]
        v = _rowsum(_sum4([(x - m) * (x - m) for x in ldx(b, c)])) * (1.0 / D)
        inv = lax.rsqrt(v + EPS)
        m = sma[pl.ds(c * RC, RC), :]
        xs = ldx(b, c)
        for i in range(4):
            hb[p][pl.ds(c * 8, 8), pl.ds(i * 128, 128)] = _pack((xs[i] - m) * inv)

    def qkv(p, n):
        y = jnp.dot(pltpu.bitcast(hb[p][...], bf16), pltpu.bitcast(wp[n], bf16), preferred_element_type=f32)
        t = n % 4
        if n < 4:
            qb[p][t] = y * QSCALE
        else:
            (kb if n < 8 else vb)[p][t, pl.ds(PAD, M), :] = y

    def halo(p, first):
        for t in range(4):
            if first:
                vb[p][t, pl.ds(0, PAD), :] = jnp.broadcast_to(vb[p][t, pl.ds(PAD, 1), :], (PAD, 128))
                kb[p][t, pl.ds(0, PAD), :] = jnp.zeros((PAD, 128), f32)
            else:
                vb[p][t, pl.ds(0, PAD), :] = vb[1 - p][t, pl.ds(M, PAD), :]
                kb[p][t, pl.ds(0, PAD), :] = kb[1 - p][t, pl.ds(M, PAD), :]

    def attn1(p, c):
        r = PAD + c * RC
        q = [qb[p][t, pl.ds(c * RC, RC), :] for t in range(4)]
        for w in range(NW):
            a = _sum4([q[t] * kb[p][t, pl.ds(r - DIL * w, RC), :] for t in range(4)])
            sl = (w, pl.ds(c * RC, RC), slice(None))
            if hops == 2:
                sa[sl] = a
                r1 = pltpu.roll(a, 64, 1)
                sb[sl] = sa[sl] + r1
            elif hops == 1:
                sa[sl] = a
                r1 = (pltpu.roll(a, 64, 1) + pltpu.roll(a, 32, 1)) + pltpu.roll(a, 96, 1)
                sb[sl] = sa[sl] + r1
            elif hops == 3:
                sb[sl] = a + pltpu.roll(a, 64, 1)
            elif hops == 4:
                sb[sl] = (a + pltpu.roll(a, 64, 1)) + (pltpu.roll(a, 32, 1) + pltpu.roll(a, 96, 1))

    def attn2(p, c, first):
        r = PAD + c * RC
        ls = []
        for w in range(NW):
            sl = (w, pl.ds(c * RC, RC), slice(None))
            if hops in (2, 3):
                r2 = pltpu.roll(sb[sl], 32, 1)
                a = sb[sl] + r2
            else:
                a = sb[sl]
            if first and c == 0 and w > 0:
                a = jnp.where(lax.broadcasted_iota(jnp.int32, (RC, 128), 0) >= DIL * w, a, NEG)
            ls.append(a)
        mx = jnp.maximum(jnp.maximum(jnp.maximum(ls[0], ls[1]), jnp.maximum(ls[2], ls[3])),
                         jnp.maximum(jnp.maximum(ls[4], ls[5]), jnp.maximum(ls[6], ls[7])))
        es = [jnp.exp2(a - mx) for a in ls]
        den = _sum4(es[:4]) + _sum4(es[4:])
        y0 = pltpu.reciprocal(den, approx=True)
        inv = y0 * (2.0 - den * y0)
        for t in range(4):
            pv = [es[w] * vb[p][t, pl.ds(r - DIL * w, RC), :] for w in range(NW)]
            ob[p][pl.ds(c * 8, 8), pl.ds(t * 128, 128)] = _pack((_sum4(pv[:4]) + _sum4(pv[4:])) * inv)

    def proj(b, p, n):
        y = jnp.dot(pltpu.bitcast(ob[p][...], bf16), pltpu.bitcast(wop[n], bf16), preferred_element_type=f32)
        x1b[n, rows(b), :] = y + xb[rows(b), pl.ds(n * 128, 128)].astype(f32)

    def ld1(b, c):
        return [x1b[i, rows(b, c * RC, RC), :] for i in range(4)]

    def ln_b(b, p, c, wr):
        xs = ld1(b, c)
        xc, inv = _ln_parts(xs)
        sc = _rowsum(_sum4([xc[i] * wr[i] for i in range(4)])) * inv
        for i in range(4):
            xo[p][pl.ds(c * RC, RC), pl.ds(i * 128, 128)] = (xs[i] + xc[i] * inv).astype(bf16)
        return [sc[:8], sc[8:]]

    def ln_b1(b, p, c):
        smb[pl.ds(c * RC, RC), :] = _rowsum(_sum4(ld1(b, c))) * (1.0 / D)

    def ln_b2(b, p, c, wr):
        m = smb[pl.ds(c * RC, RC), :]
        xc = [x - m for x in ld1(b, c)]
        v = _rowsum(_sum4([x * x for x in xc])) * (1.0 / D)
        sc = _rowsum(_sum4([xc[i] * wr[i] for i in range(4)]))
        inv = lax.rsqrt(v + EPS)
        sc = sc * inv
        m = smb[pl.ds(c * RC, RC), :]
        xs = ld1(b, c)
        for i in range(4):
            xo[p][pl.ds(c * RC, RC), pl.ds(i * 128, 128)] = (xs[i] + (xs[i] - m) * inv).astype(bf16)
        return [sc[:8], sc[8:]]

    def merge_lanes(vs, shift=0):
        lane = _lane_iota(8)
        bit = shift
        while len(vs) > 1:
            msk = ((lane >> bit) & 1) == 1
            vs = [jnp.where(msk, vs[2 * k + 1], vs[2 * k]) for k in range(len(vs) // 2)]
            bit += 1
        return vs[0]

    def load_wr():
        w = wr_v[...].astype(f32).reshape(1, D)
        return [jnp.broadcast_to(w[:, i * 128:(i + 1) * 128], (RC, 128)) for i in range(4)]

    def step(i, p, do_lna, do_qkv, do_attn, do_proj, first_attn=False, first_qkv=False):
        ev = []

        def at(t, f):
            ev.append((t, len(ev), f))
        nm = (4 if do_proj else 0) + (12 if do_qkv else 0)
        k = 0
        if do_proj:
            for n in range(4):
                at(k / nm, functools.partial(proj, i - 2, p, n))
                k += 1
        t_proj = k / nm
        if do_qkv:
            if not first_qkv:
                at(0, functools.partial(halo, p, False))
            for n in range(12):
                at(k / nm, functools.partial(qkv, p, n))
                k += 1
            if first_qkv:
                at(1.5, functools.partial(halo, p, True))
        slots = NCH + lag
        for c in range(NCH):
            if do_attn:
                at(c / slots, functools.partial(attn1, 1 - p, c))
                at((c + lag) / slots, functools.partial(attn2, 1 - p, c, first_attn))
            if do_lna:
                if stage_ln:
                    at(c / slots, functools.partial(ln_a1, i + 1, 1 - p, c))
                    at((c + lag) / slots, functools.partial(ln_a2, i + 1, 1 - p, c))
                else:
                    at(c / NCH, functools.partial(ln_a, i + 1, 1 - p, c))
        scores = []
        if do_proj:
            wr = load_wr()
            span = max(1 - t_proj, 0.01)
            for c in range(NCH):
                if stage_ln:
                    at(t_proj + span * c / slots, functools.partial(ln_b1, i - 2, p, c))
                    at(t_proj + span * (c + lag) / slots, lambda c=c: scores.extend(ln_b2(i - 2, p, c, wr)))
                else:
                    at(t_proj + span * c / NCH, lambda c=c: scores.extend(ln_b(i - 2, p, c, wr)))
        for _, _, f in sorted(ev, key=lambda e: e[:2]):
            f()
        if do_proj:
            rb[i - 2] = merge_lanes(scores)

    def route_ffn():
        RV = M // 8
        G = 128 // RV
        sh = RV.bit_length() - 1
        sc = jnp.concatenate([merge_lanes([rb[a * G + k] for k in range(G)], sh) for a in range(NB // G)], axis=0)
        row = lax.broadcasted_iota(jnp.int32, sc.shape, 0)
        lane = lax.broadcasted_iota(jnp.int32, sc.shape, 1)
        pos = (row >> 3) * 1024 + lane * 8 + (row & 7)
        sc = jnp.where(sc == sc, sc, -jnp.inf)
        m1 = jnp.max(sc)
        i1 = jnp.min(jnp.where(sc == m1, pos, S))
        sc2 = jnp.where(pos == i1, -jnp.inf, sc)
        m2 = jnp.max(sc2)
        i2 = jnp.min(jnp.where((sc2 == m2) & (pos != i1), pos, S))
        idx = [jnp.clip(i1, 0, S - 1), jnp.clip(i2, 0, S - 1)]
        first = lax.broadcasted_iota(jnp.int32, (16, 128), 0) < 8
        xs = [jnp.where(first, jnp.broadcast_to(x1b[i, pl.ds(idx[0], 1), :], (16, 128)),
                        jnp.broadcast_to(x1b[i, pl.ds(idx[1], 1), :], (16, 128))) for i in range(4)]
        xc, inv = _ln_parts(xs)
        hsel = jnp.concatenate([c * inv for c in xc], axis=1).astype(bf16)
        nt = (((1,), (1,)), ((), ()))
        g = lax.dot_general(hsel, wg_v[...], nt, preferred_element_type=f32)
        u = lax.dot_general(hsel, wu_v[...], nt, preferred_element_type=f32)
        act = (g * jax.nn.sigmoid(g) * u).astype(bf16)
        y = jnp.dot(act, wd_v[...], preferred_element_type=f32)
        gate = jax.nn.sigmoid(jnp.where(first, m1, m2))
        upd = [y[:, i * 128:(i + 1) * 128] * gate for i in range(4)]
        bases = [pl.multiple_of((idx[k] >> 4) << 4, 16) for k in range(2)]
        rowi = lax.broadcasted_iota(jnp.int32, (16, 128), 0)
        for k in range(2):
            xs = [x1b[i, pl.ds(bases[k], 16), :] for i in range(4)]
            xc, inv = _ln_parts(xs)
            hit0 = rowi + bases[k] == idx[0]
            hit1 = rowi + bases[k] == idx[1]
            for i in range(4):
                u0 = jnp.broadcast_to(upd[i][0:1], (16, 128))
                u1 = jnp.broadcast_to(upd[i][8:9], (16, 128))
                add = jnp.where(hit0, u0, jnp.where(hit1, u1, 0.0))
                fix[k, :, pl.ds(i * 128, 128)] = (xs[i] + (xc[i] * inv + add)).astype(bf16)
        return bases

    def when(cond, f):
        if isinstance(cond, bool):
            if cond:
                f()
        else:
            pl.when(cond)(f)

    if only_body:
        def body(j, c):
            step(2 * j, 0, True, True, True, True)
            o_copy(0, 0).start()
            o_copy(0, 0).wait()
            step(2 * j + 1, 1, True, True, True, True)
            return c
        lax.fori_loop(1, 3, body, 0)
        return

    w_copy(0).start()
    x_copy(0).start()
    w_copy(1).start()
    w_copy(2).start()
    x_copy(1).start()
    wo_copy.start()
    wr_copy.start()
    for b in range(2, NB):
        x_copy(b).start()
    wg_copy.start()
    wu_copy.start()
    wd_copy.start()
    for j in range(3):
        w_copy(j).wait()
        permute_w(j)
    wo_copy.wait()
    permute_wo()
    wr_copy.wait()

    def layer(l):
        def full(i, p, lna, qkv_, attn):
            if lna:
                when(l == 0, lambda: x_copy(i + 1).wait())
            when(i >= 4, lambda: o_copy(0, p).wait())
            step(i, p, lna, qkv_, attn, True)
            when(l == 0, lambda: r_copy(i - 2, p).start())
            when(l == 1, lambda: o_copy(i - 2, p).start())

        def pre():
            x_copy(0).wait()
            x_copy(1).wait()
            x_copy(2).wait()
        when(l == 0, pre)
        for c in range(NCH):
            ln_a(0, 0, c)
        step(0, 0, True, True, False, False, first_qkv=True)
        step(1, 1, True, True, True, False, first_attn=True)

        def body(j, c):
            full(2 * j, 0, True, True, True)
            full(2 * j + 1, 1, True, True, True)
            return c
        lax.fori_loop(1, NB // 2 - 1, body, 0)
        full(NB - 2, 0, True, True, True)
        full(NB - 1, 1, False, True, True)
        full(NB, 0, False, False, True)
        full(NB + 1, 1, False, False, False)

        def wait_ffn():
            wg_copy.wait()
            wu_copy.wait()
            wd_copy.wait()
        when(l == 0, wait_ffn)
        bases = route_ffn()
        o_copy(0, 0).wait()
        o_copy(0, 1).wait()

        def mid():
            for k in range(2):
                xb[pl.ds(bases[k], 16), :] = fix[k]
        when(l == 0, mid)

        def final():
            cps = [pltpu.make_async_copy(fix.at[k], out_hbm.at[0, pl.ds(bases[k], 16)], sem_o.at[k]) for k in range(2)]
            cps[0].start()

            @pl.when(bases[0] != bases[1])
            def _():
                cps[1].start()
                cps[1].wait()
            cps[0].wait()
        when(l == 1, final)

    lax.fori_loop(0, 2, lambda l, c: (layer(l), c)[1], 0)


def build(M=256, hops=2, lag=1, only_body=False, stage_ln=True, flags=None):
    NB = S // M
    V = pltpu.VMEM

    def fn(A_x, A_wqkv, A_wo, B_x, B_w_r, B_w_gate, B_w_up, B_w_down):
        del B_x
        any_spec = pl.BlockSpec(memory_space=pltpu.MemorySpace.HBM)
        return pl.pallas_call(
            functools.partial(_kernel, M=M, hops=hops, lag=lag, only_body=only_body, stage_ln=stage_ln),
            out_shape=jax.ShapeDtypeStruct((1, S, D), bf16),
            in_specs=[any_spec] * 7,
            out_specs=any_spec,
            scratch_shapes=[
                V((S, D), bf16), V((3, D, D), bf16), V((12, D // 2, 128), u32),
                V((D, D), bf16), V((4, D, 128), f32), V((4, D // 2, 128), u32),
                V((D,), bf16), V((F, D), bf16), V((F, D), bf16), V((F, D), bf16),
                V((M // 2, D), u32), V((M // 2, D), u32),
                V((4, M, 128), f32), V((4, M, 128), f32),
                V((4, M + PAD, 128), f32), V((4, M + PAD, 128), f32),
                V((4, M + PAD, 128), f32), V((4, M + PAD, 128), f32),
                V((M // 2, D), u32), V((M // 2, D), u32),
                V((M, D), bf16), V((M, D), bf16),
                V((4, S, 128), f32), V((NB, 8, 128), f32),
                V((NW, M, 128), f32), V((NW, M, 128), f32), V((NW, M, 128), f32),
                V((M, 128), f32), V((M, 128), f32), V((2, 16, D), bf16),
                pltpu.SemaphoreType.DMA((NB,)), pltpu.SemaphoreType.DMA((8,)), pltpu.SemaphoreType.DMA((2,)),
            ],
            compiler_params=pltpu.CompilerParams(vmem_limit_bytes=100 * 1024 * 1024, flags=flags),
        )(A_x, A_wqkv, A_wo, B_w_r, B_w_gate.T, B_w_up.T, B_w_down)
    return fn


_fn = build(M=256, hops=3, lag=1)


@jax.jit
def pallas_interleave_layers__sliding_local_dilated__moe_arch_mod__prompt_kernel(
    A_x, A_wqkv, A_wo, B_x, B_w_r, B_w_gate, B_w_up, B_w_down
):
    return _fn(A_x, A_wqkv, A_wo, B_x, B_w_r, B_w_gate, B_w_up, B_w_down)
```

```python
import contextlib
import functools
import numpy as np
import jax
import jax.numpy as jnp
from jax import lax
import jax.experimental.pallas as pl
import jax.experimental.pallas.tpu as pltpu

S, D, F = 2048, 512, 1376
NW, DIL = 8, 2
PAD = 16
RC = 16
RA = 8
HS = 17
LOG2E = 1.4426950408889634
QSCALE = 0.25 * LOG2E
NEG = -1e9 * LOG2E
EPS = 1e-5
f32, bf16, u32 = jnp.float32, jnp.bfloat16, jnp.uint32


def _lane_iota(rows):
    return lax.broadcasted_iota(jnp.int32, (rows, 128), 1)


def _row_iota(rows):
    return lax.broadcasted_iota(jnp.int32, (rows, 128), 0)


def _sum4(a):
    return (a[0] + a[1]) + (a[2] + a[3])


def _rowsum(x):
    return jnp.broadcast_to(jnp.sum(x, axis=1, keepdims=True), x.shape)


def _pack(x):
    return pltpu.bitcast(x.astype(bf16), u32)


def _inv_std(xc):
    return lax.rsqrt(_rowsum(_sum4([x * x for x in xc])) * (1.0 / D) + EPS)


def _cols(i):
    return pl.ds(i * 128, 128)


def _kernel(x_hbm, wqkv_hbm, wo_hbm, wr_hbm, wg_hbm, wu_hbm, wd_hbm, out_hbm,
            xb, wraw, wp, woraw, wof, wop, wr_v, wg_v, wu_v, wd_v,
            hb0, hb1, qb0, qb1, kb0, kb1, vb0, vb1, ob0, ob1, x1b, mb, ib, rb, fix, wt, lg,
            sem_x, sem_w, sem_o, sem_q, *, M, c):
    NB = S // M
    NCH = M // RC
    hb, qb, kb, vb, ob = (hb0, hb1), (qb0, qb1), (kb0, kb1), (vb0, vb1), (ob0, ob1)
    scope = jax.named_scope if c["scopes"] else (lambda n: contextlib.nullcontext())

    def rows(b, off=0, n=M):
        if isinstance(b, int):
            return pl.ds(b * M + off, n)
        return pl.ds(pl.multiple_of(b * M + off, RC), n)

    def x_copy(b0, b1):
        r = pl.ds(b0 * M, (b1 - b0) * M)
        return pltpu.make_async_copy(x_hbm.at[0, r], xb.at[r], sem_x.at[b0])

    def o_copy(b):
        return pltpu.make_async_copy(xb.at[rows(b)], out_hbm.at[0, rows(b)], sem_o.at[b])

    def w_copy(j):
        return pltpu.make_async_copy(wqkv_hbm.at[:, pl.ds(j * D, D)], wraw.at[j], sem_w.at[j])

    def wq_copy(k, n):
        r = pl.ds(k * D // n, D // n)
        return pltpu.make_async_copy(wqkv_hbm.at[r, pl.ds(0, D)], wraw.at[0, r], sem_q.at[k])

    def wo_copy():
        return pltpu.make_async_copy(wo_hbm, woraw, sem_w.at[3])

    def wr_copy():
        return pltpu.make_async_copy(wr_hbm, wr_v, sem_w.at[4])

    def ffn_copy(k):
        s, d = ((wg_hbm, wg_v), (wu_hbm, wu_v), (wd_hbm, wd_v))[k]
        return pltpu.make_async_copy(s, d, sem_w.at[5 + k])

    def permute_w(j, r, R):
        lane = _lane_iota(R)
        c0 = ((lane >> 2) & 1) == 1
        c1 = ((lane >> 3) & 1) == 1
        a = [pltpu.bitcast(wraw[j, pl.ds(2 * r, 2 * R), _cols(i)], u32) for i in range(4)]
        b = [jnp.where(c0, a[i ^ 1], a[i]) for i in range(4)]
        m = [jnp.where(c1, b[i ^ 2], b[i]) for i in range(4)]
        for t in range(4):
            idx = (lane & 7) * 16 + (((lane >> 3) & 3) ^ t) * 4 + (lane >> 5)
            wp[j * 4 + t, pl.ds(r, R), :] = jnp.take_along_axis(m[t], idx, axis=1)

    def widen_wo(n):
        for h in range(32):
            i = h >> 3
            w = woraw[pl.ds(h * 16, 16), _cols(n)].astype(f32)
            for half in range(2):
                part = w[8 * half:8 * half + 8]
                if i & 1:
                    part = pltpu.roll(part, 4, 0)
                wof[n, pl.ds(h * HS + 8 * (half ^ (i >> 1)), 8), :] = part

    def permute_wo(n):
        for e in range(16):
            for m in range(2):
                lo = wof[n, pl.ds(16 * m * HS + e, 8, stride=2 * HS), :]
                hi = wof[n, pl.ds((16 * m + 1) * HS + e, 8, stride=2 * HS), :]
                wop[n, pl.ds(e * 16 + m * 8, 8), :] = (pltpu.bitcast(lo, u32) >> 16) | pltpu.bitcast(hi, u32)

    carry = {}

    def tsum(a, chain):
        if chain:
            return functools.reduce(lambda x, y: x + y, a)
        return a[0] if len(a) == 1 else tsum(a[:len(a) // 2], 0) + tsum(a[len(a) // 2:], 0)

    def ldx(sl):
        return [xb[sl, _cols(i)].astype(f32) for i in range(4)]

    def hbuf(b, p):
        return ob[1] if isinstance(b, int) and b == 0 else hb[p]

    def ln_a1(b, p, k):
        carry["a", b if isinstance(b, int) else 0, k] = _rowsum(_sum4(ldx(rows(b, k * RC, RC)))) * (1.0 / D)

    def ln_a2(b, p, k):
        m = carry.pop(("a", b if isinstance(b, int) else 0, k))
        xc = [x - m for x in ldx(rows(b, k * RC, RC))]
        inv = _inv_std(xc)
        for i in range(4):
            hbuf(b, p)[pl.ds(k * 8, 8), _cols(i)] = _pack(xc[i] * inv)

    def put_qkv(y, p, n, r, nr):
        t = n % 4
        if n < 4:
            qb[p][t, pl.ds(r, nr), :] = y * QSCALE
        else:
            (kb if n < 8 else vb)[p][t, pl.ds(r + PAD, nr), :] = y

    def qkv(p, n, b=None):
        y = jnp.dot(pltpu.bitcast(hbuf(b, p)[...], bf16), pltpu.bitcast(wp[n], bf16), preferred_element_type=f32)
        put_qkv(y, p, n, 0, M)

    def halo(b, p, do_k=True, do_v=True):
        for t in range(4):
            if do_k:
                if isinstance(b, int) and b == 0:
                    kb[p][t, pl.ds(0, PAD), :] = jnp.zeros((PAD, 128), f32)
                else:
                    kb[p][t, pl.ds(0, PAD), :] = kb[1 - p][t, pl.ds(M, PAD), :]
            if do_v:
                v0 = jnp.broadcast_to(vb[p][t, pl.ds(PAD, 1), :], (PAD, 128))
                if isinstance(b, int):
                    vb[p][t, pl.ds(0, PAD), :] = v0 if b == 0 else vb[1 - p][t, pl.ds(M, PAD), :]
                else:
                    vb[p][t, pl.ds(0, PAD), :] = jnp.where(b == 0, v0, vb[1 - p][t, pl.ds(M, PAD), :])

    def attn1(p, r, key, nr):
        q = [qb[p][t, pl.ds(r, nr), :] for t in range(4)]
        out = []
        for w in range(NW):
            a = tsum([q[t] * kb[p][t, pl.ds(r + (PAD - DIL * w), nr), :] for t in range(4)], c["ch"] & 1)
            out.append(a + pltpu.roll(a, 64, 1))
        carry["t", key] = out

    def attn2(p, r, key, nr, pos0, dst=None, park=False):
        ls = []
        for w, a in enumerate(carry.pop(("t", key))):
            a = a + pltpu.roll(a, 32, 1)
            if w > 0 and pos0 is not None:
                a = jnp.where(_row_iota(nr) + pos0 >= DIL * w, a, NEG)
            ls.append(a)
        if park:
            for w in range(NW):
                lg[w, pl.ds(r, nr), :] = ls[w]
        else:
            attn3(p, r, key, nr, dst, ls)

    def attn3(p, r, key, nr, dst=None, ls=None):
        if ls is None:
            ls = [lg[w, pl.ds(r, nr), :] for w in range(NW)]
        mx = jnp.maximum(jnp.maximum(jnp.maximum(ls[0], ls[1]), jnp.maximum(ls[2], ls[3])),
                         jnp.maximum(jnp.maximum(ls[4], ls[5]), jnp.maximum(ls[6], ls[7])))
        es = [jnp.exp2(a - mx) for a in ls]
        den = _sum4(es[:4]) + _sum4(es[4:])
        y0 = pltpu.reciprocal(den, approx=True)
        inv = y0 * (2.0 - den * y0)
        res = []
        for t in range(4):
            pv = [es[w] * vb[p][t, pl.ds(r + (PAD - DIL * w), nr), :] for w in range(NW)]
            res.append(tsum(pv, c["ch"] & 2) * inv)
        if nr == 8:
            if key % 2 == 0:
                carry["o"] = res
                return
            res = [jnp.concatenate([a, b], axis=0) for a, b in zip(carry.pop("o"), res)]
            r = r - 8
        r2 = r // 2 if isinstance(r, int) else pl.multiple_of(r >> 1, 8)
        for t in range(4):
            (ob[p] if dst is None else dst)[pl.ds(r2, 8), _cols(t)] = _pack(res[t])

    def proj(b, p, n, off=0, nr=M, src=None):
        sl = pl.ds(off // 2, nr // 2)
        o = pltpu.bitcast((ob[p] if src is None else src)[sl, :], bf16)
        y = jnp.dot(o, pltpu.bitcast(wop[n], bf16), preferred_element_type=f32)
        x1b[n, rows(b, off, nr), :] = y + xb[rows(b, off, nr), _cols(n)].astype(f32)

    def ld1(sl):
        return [x1b[i, sl, :] for i in range(4)]

    def ln_b1(b, p, k):
        carry["b", p, k] = _rowsum(_sum4(ld1(rows(b, k * RC, RC)))) * (1.0 / D)

    def ln_b2(b, p, k, split=False):
        sl = rows(b, k * RC, RC)
        m = carry.pop(("b", p, k))
        xs = ld1(sl)
        xc = [x - m for x in xs]
        wr = carry["wr"]
        var = _rowsum(_sum4([x * x for x in xc]))
        dot = _rowsum(_sum4([xc[i] * wr[i] for i in range(4)]))
        mb[sl, :] = m
        if split:
            carry["b3", p, k] = (m, var, dot)
            return
        inv = lax.rsqrt(var * (1.0 / D) + EPS)
        ln_b_out(b, p, k, [xs[i] + xc[i] * inv for i in range(4)], inv, dot)

    def ln_b3(b, p, k):
        m, var, dot = carry.pop(("b3", p, k))
        inv = lax.rsqrt(var * (1.0 / D) + EPS)
        gain, off = inv + 1.0, m * inv
        ln_b_out(b, p, k, [x * gain - off for x in ld1(rows(b, k * RC, RC))], inv, dot)

    def ln_b_out(b, p, k, ys, inv, dot):
        sl = rows(b, k * RC, RC)
        ib[sl, :] = inv
        for i in range(4):
            xb[sl, _cols(i)] = ys[i].astype(bf16)
        sc = dot * inv
        lane = _lane_iota(8)
        pair = jnp.where((lane & 1) == 1, sc[8:], sc[:8])
        if k == 0:
            carry["sc", p] = pair
        else:
            carry["sc", p] = jnp.where(((lane >> 1) & (NCH - 1)) == k, pair, carry["sc", p])
        if k == NCH - 1:
            rb[b] = carry.pop(("sc", p))

    def load_wr():
        w = wr_v[...].astype(f32).reshape(1, D)
        carry["wr"] = [jnp.broadcast_to(w[:, i * 128:(i + 1) * 128], (RC, 128)) for i in range(4)]

    class Plan:
        def __init__(self):
            self.ev = []

        def at(self, t, f, *a):
            self.ev.append((t, len(self.ev), functools.partial(f, *a)))

        def staged(self, span, n, lag, fs, k0=0):
            dt = (span[1] - span[0]) / (n + lag * (len(fs) - 1))
            for k in range(n):
                for s, f in enumerate(fs):
                    self.at(span[0] + (k + s * lag) * dt + 1e-6, f, k0 + k)

        def ln_a(self, span, b, p, lag=c["lag"]):
            self.staged(span, NCH, lag, [functools.partial(f, b, p) for f in (ln_a1, ln_a2)])

        def ln_b(self, span, b, p, k0=0, n=NCH, lag=c["lagb"], three=c["b3"]):
            fs = (ln_b1, functools.partial(ln_b2, split=True), ln_b3) if three else (ln_b1, ln_b2)
            self.staged(span, n, lag, [functools.partial(f, b, p) for f in fs], k0)

        def attn(self, span, b, p, lag=c["laga"], dst=None, park=False, k0=0, n=M // RA):
            def second(k):
                masked = k * RA < DIL * (NW - 1) and not (isinstance(b, int) and b > 0)
                attn2(p, k * RA, k, RA, b * M + k * RA if masked else None, dst, park)
            self.staged(span, n, lag, [lambda k: attn1(p, k * RA, k, RA), second], k0)

        def attn_rest(self, span, p, n, dst=None):
            self.staged(span, n, 0, [lambda k: attn3(p, k * RA, k, RA, dst)])

        def run(self):
            for _, _, f in sorted(self.ev, key=lambda e: e[:2]):
                f()

    def step(j, p):
        def blk(o):
            return (j + o) & (NB - 1)
        pn = Plan()
        pl.when(j > NB + 2)(lambda: o_copy(j - 3 - NB).start())
        for k in range(3):
            if (3 + k) % 2 == p:
                pl.when(j == 3 + k)(lambda k=k: ffn_copy(k).start())
        load_wr()
        for n in range(4):
            pn.at((n + c['sh']) / 16, proj, blk(-2), p, n)
        for n in range(12):
            pn.at((4 + n + c['sh']) / 16, qkv, p, n)
        pn.at(2.0, halo, blk(0), p)
        pn.attn(c["sa"], blk(-1), 1 - p)
        pn.ln_a(c["sl"], blk(1), 1 - p)
        pn.ln_b(c["sb"], blk(-2), p)
        pn.run()

    def last_qkv():
        pn = Plan()
        for n in range(12):
            pn.at(n / 12, qkv, 1, n)
        pn.at(0, halo, NB - 1, 1, True, False)
        pn.at(2.0, halo, NB - 1, 1, False, True)
        pn.attn((0, c["e1"][0]), NB - 2, 0, c["e1"][1])
        if c["ne"]:
            pn.attn((max(c["e1"][0], 0.6), 1), NB - 1, 1, c["e1"][2], park=True, n=c["ne"])
        pn.run()

    def drain():
        pn = Plan()
        load_wr()
        t = c["dr"]
        for n in range(4):
            pn.at(n * M, proj, NB - 3, 1, n)
            pn.at((4 + n) * M, proj, NB - 2, 0, n)
        if c["ne"]:
            pn.attn_rest((0, t[3]), 1, c["ne"], hb[0])
        if c["ne"] < M // RA:
            pn.attn((t[3], t[0]), NB - 1, 1, c["dlag"][0], hb[0], k0=c["ne"], n=M // RA - c["ne"])
        pn.ln_b(t[1], NB - 3, 0, lag=c["dlag"][1], three=c["d3"])
        pn.ln_b(t[2], NB - 2, 1, lag=c["dlag"][2], three=c["d3"])
        t0, off = 8 * M, 0
        for nr, span in c["parts"]:
            for n in range(4):
                pn.at(t0 + n * nr, proj, NB - 1, 1, n, off, nr, hb[0])
            pn.ln_b(span, NB - 1, 2, off // RC, nr // RC, c["dlag"][3], c["d3"])
            t0, off = t0 + 4 * nr, off + nr
        pn.run()

    def merge_lanes(vs, bit):
        lane = _lane_iota(8)
        while len(vs) > 1:
            msk = ((lane >> bit) & 1) == 1
            vs = [jnp.where(msk, vs[2 * k + 1], vs[2 * k]) for k in range(len(vs) // 2)]
            bit += 1
        return vs[0]

    def route_ffn():
        NT = c["NT"]

        def flip():
            for i in range(NT):
                for k, w in enumerate((wg_v, wu_v)):
                    r0 = F - (F % 128) - 128 * (NT - i)
                    for t in range(4):
                        wt[2 * i + k, pl.ds(64 * t, 64), :] = pltpu.bitcast(w[pl.ds(r0, 128), _cols(t)].T, u32)
        if c["flip_first"]:
            flip()
        RV = M // 8
        G = 128 // RV
        sh = RV.bit_length() - 1
        sc = jnp.concatenate([merge_lanes([rb[a * G + k] for k in range(G)], sh) for a in range(NB // G)], axis=0)
        row = _row_iota(16)
        pos = (row >> 3) * 1024 + _lane_iota(16) * 8 + (row & 7)
        bits = pltpu.bitcast(jnp.where(sc == 0.0, 0.0, sc), jnp.int32)
        mono = bits ^ ((bits >> 31) & 0x7FFFFFFF)
        mono = jnp.where(sc == sc, mono, -0x80000000)
        key = pltpu.bitcast((((mono >> 2) + 0x20800000) & ~(S - 1)) | (S - 1 - pos), f32)

        def top(k):
            return jnp.max(jnp.max(k, axis=0, keepdims=True), axis=1, keepdims=True)
        k1 = top(key)
        k2 = top(jnp.where(key == k1, 0.0, key))
        idx = [(S - 1) - (pltpu.bitcast(k, jnp.int32)[0, 0] & (S - 1)) for k in (k1, k2)]
        first = row < 8
        if not c["flip_first"]:
            flip()

        def pick(ref, *lead):
            a, b = [jnp.broadcast_to(ref[(*lead, pl.ds(i, 1), slice(None))], (16, 128)) for i in idx]
            return jnp.where(first, a, b)
        m, inv = pick(mb), pick(ib)
        hs = [(pick(x1b, i) - m) * inv for i in range(4)]
        hsel = jnp.concatenate(hs, axis=1).astype(bf16)
        nt = (((1,), (1,)), ((), ()))
        cut = F - (F % 128) - 128 * NT
        last = F - (F % 128)

        def proj_in(k, w):
            parts = [lax.dot_general(hsel, w[pl.ds(0, cut), :], nt, preferred_element_type=f32)] if cut else []
            tail = lax.dot_general(hsel, w[pl.ds(last, F - last), :], nt, preferred_element_type=f32)
            return parts, tail
        (g0, gt), (u0, ut) = proj_in(0, wg_v), proj_in(1, wu_v)

        def act(g, u):
            return (g * jax.nn.sigmoid(g) * u).astype(bf16)
        acts = [act(g, u) for g, u in zip(g0, u0)]
        for i in range(NT):
            g, u = [jnp.dot(hsel, pltpu.bitcast(wt[2 * i + k], bf16), preferred_element_type=f32) for k in range(2)]
            acts.append(act(g, u))
        y = jnp.dot(act(gt, ut), wd_v[pl.ds(last, F - last), :], preferred_element_type=f32)
        y = y + jnp.dot(jnp.concatenate(acts, axis=1), wd_v[pl.ds(0, last), :], preferred_element_type=f32)
        load_wr()
        gate = jax.nn.sigmoid(_rowsum(_sum4([hs[i] * carry["wr"][i] for i in range(4)])))
        upd = [y[:, i * 128:(i + 1) * 128] * gate for i in range(4)]
        bases = [pl.multiple_of(i & ~15, 16) for i in idx]
        for k in range(2):
            sl = pl.ds(bases[k], 16)
            xs, m, inv = ld1(sl), mb[sl, :], ib[sl, :]
            hit0 = row + bases[k] == idx[0]
            hit1 = row + bases[k] == idx[1]
            for i in range(4):
                u0 = jnp.concatenate([upd[i][:8]] * 2, axis=0)
                u1 = jnp.concatenate([upd[i][8:]] * 2, axis=0)
                add = jnp.where(hit0, u0, jnp.where(hit1, u1, 0.0))
                fix[pl.ds(16 * k, 16), _cols(i)] = (xs[i] + ((xs[i] - m) * inv + add)).astype(bf16)
        return bases

    def mid_fixup(bases):
        for k in range(2):
            xb[pl.ds(bases[k], 16), :] = fix[pl.ds(16 * k, 16), :]

        def one(k, z):
            base = jnp.where(k == 0, bases[0], bases[1])
            r = pl.multiple_of(base & (M - 1), 16)

            @pl.when(base < 3 * M)
            def _():
                xs = ldx(pl.ds(pl.multiple_of(base, 16), 16))
                m = _rowsum(_sum4(xs)) * (1.0 / D)
                xc = [x - m for x in xs]
                inv = _inv_std(xc)
                h = jnp.concatenate([x * inv for x in xc], axis=1).astype(bf16)

                @pl.when(base >= 2 * M)
                def _():
                    hb[0][pl.ds(pl.multiple_of(r >> 1, 8), 8), :] = pltpu.bitcast(h, u32)

                @pl.when(base < 2 * M)
                def _():
                    ys = [jnp.dot(h, pltpu.bitcast(wp[n], bf16), preferred_element_type=f32) for n in range(12)]
                    for p in range(2):
                        @pl.when((base >= M) == (p == 1))
                        def _():
                            for n in range(12):
                                put_qkv(ys[n], p, n, r, 16)

                @pl.when(base < M)
                def _():
                    halo(0, 0)
                    halo(1, 1)
                    rs = [r, pl.multiple_of(jnp.minimum(r + 16, M - 16), 16)]
                    for q in range(2):
                        attn1(0, rs[q], ("redo", q), 16)
                    for q in range(2):
                        attn2(0, rs[q], ("redo", q), 16, rs[q])
            return z
        lax.fori_loop(0, 2, one, 0)

    def final_fixup(bases):
        for b in range(NB):
            o_copy(b).wait()
        cps = [pltpu.make_async_copy(fix.at[pl.ds(16 * k, 16)], out_hbm.at[0, pl.ds(bases[k], 16)], sem_o.at[k])
               for k in range(2)]
        cps[0].start()

        @pl.when(bases[0] != bases[1])
        def _():
            cps[1].start()
            cps[1].wait()
        cps[0].wait()

    XC = c["XC"]
    PR = c["PR"]
    NP = D // 2 // PR

    def p3():
        pn = Plan()
        for n in range(2):
            pn.at(n, qkv, 1, n)
        for n in range(4):
            pn.at(2 + n, qkv, 0, 4 + n, 0)
        for k in range(NP):
            pn.at(1.5 * k / NP, permute_w, 1, PR * k, PR)
        pn.at(9, halo, 0, 0, True, False)
        pn.run()

    def p4():
        pn = Plan()
        for k in range(NP):
            pn.at(1.5 * k / NP, permute_w, 2, PR * k, PR)
        for n in range(2):
            pn.at(n, qkv, 1, 2 + n)
        for n in range(4):
            pn.at(2 + n, qkv, 0, 8 + n, 0)
        pn.at(7, halo, 0, 0, False, True)
        pn.ln_a(c["p4l"], 2, 0, c["p4lag"][0])
        if c["np"]:
            pn.attn(c["p4q"], 0, 0, c["p4lag"][2], park=True, n=c["np"])
        pn.run()

    def p5():
        pn = Plan()
        for n in range(4):
            pn.at(n, qkv, 1, 4 + n)
            pn.at(4 + n, qkv, 1, 8 + n)
            pn.at(c["p4w"][0] + n * c["p4w"][1], widen_wo, n)
            pn.at(c["p4w"][0] + (n + 1.5) * c["p4w"][1], permute_wo, n)
        pn.at(15, halo, 1, 1)
        if c["np"]:
            pn.attn_rest((0, c["p4a"][0]), 0, c["np"])
        if c["np"] < M // RA:
            pn.attn(c["p4a"], 0, 0, c["p4lag"][1], k0=c["np"], n=M // RA - c["np"])
        pn.run()

    if c["only_body"]:
        part = dict(step=lambda j: step(j, 0), drain=lambda j: drain(), e1=lambda j: last_qkv(), p3=lambda j: p3(), p4=lambda j: p4(), p5=lambda j: p5(),
                    ffn=lambda j: route_ffn())[c["part"]]
        def run_part(j, z):
            carry["zero"] = j >> 20
            part(j)
            return z
        lax.fori_loop(2, 2 + c["only_body"], run_part, 0)
        for ref in hb + qb + kb + vb + ob + (xb, x1b, rb, mb, ib, wop, wp, fix, wt, lg):
            cp = pltpu.make_async_copy(ref, ref, sem_o.at[0])
            cp.start()
            cp.wait()
        return

    x_copy(0, 1).start()
    for k in range(c["QS"]):
        wq_copy(k, c["QS"]).start()
    x_copy(1, 2).start()
    with scope("p0"):
        x_copy(0, 1).wait()
        pn = Plan()
        pn.ln_a((0, 1), 0, 0, 3)
        pn.run()
    with scope("p1"):
        w_copy(1).start()
        for k in range(NP):
            if k % (NP // c["QS"]) == 0:
                wq_copy(k // (NP // c["QS"]), c["QS"]).wait()
            permute_w(0, PR * k, PR)
    with scope("p2"):
        x_copy(2, 3).start()
        w_copy(2).start()
        x_copy(1, 2).wait()
        pn = Plan()
        for n in range(4):
            pn.at(n / 4, qkv, 0, n, 0)
        pn.ln_a((0, 0.8), 1, 1, 2)
        pn.run()
    with scope("p3"):
        wo_copy().start()
        wr_copy().start()
        w_copy(1).wait()
        p3()
    with scope("p4"):
        x_copy(3, XC).start()
        x_copy(2, 3).wait()
        w_copy(2).wait()
        p4()
    with scope("p5"):
        wo_copy().wait()
        wr_copy().wait()
        p5()
        x_copy(3, XC).wait()

    def layer(l, z):
        def body(j, z2):
            with scope("body"):
                for p in range(2):
                    pl.when((j & 1) == p)(functools.partial(step, j, p))
            return z2
        lax.fori_loop(2 + l * NB, NB + 2 + l * (NB - 3), body, 0)

        @pl.when(l == 1)
        def _():
            with scope("e1"):
                o_copy(NB - 4).start()
                last_qkv()

        @pl.when(l > c["one"])
        def _():
            carry["zero"] = l >> 4
            with scope("drain"):
                drain()
                for b in range(NB - 3, NB):
                    o_copy(b).start()

        @pl.when(l == 0)
        def _():
            for k in range(3):
                ffn_copy(k).wait()
        with scope("ffn"):
            bases = route_ffn()
        with scope("fixup"):
            pl.when(l == 0)(lambda: mid_fixup(bases))
            pl.when(l == 1)(lambda: final_fixup(bases))
        return z
    lax.fori_loop(0, 2, layer, 0)


DEFAULT = dict(only_body=False, part='step', scopes=False, one=0, XC=8, QS=2, prio=0, PR=64, NT=5, flip_first=True,
               sa=(0.01, 1.0), sl=(0.04, 0.44), sb=(0.45, 0.96), lag=1, lagb=1.2, laga=1.3, ch=3, sh=0, b3=False,
               ne=0, e1=(1.0, 1.3, 2), dr=(1622.0, (1484.0, 2253.0), (2263.0, 2561.0), 0), dlag=(3.5, 2, 4, 4),
               parts=((192, (2850, 3150)), (64, (3200, 3400))), d3=True,
               p4w=(0.26, 1.03), p4a=(0.05, 7.21), p4lag=(1, 3, 2), p4l=(0.84, 5.77), np=0, p4q=(2, 6))


def build(M=256, flags=None, **kw):
    NB = S // M
    V = pltpu.VMEM
    c = dict(DEFAULT, **kw)

    def fn(A_x, A_wqkv, A_wo, B_x, B_w_r, B_w_gate, B_w_up, B_w_down):
        del B_x
        any_spec = pl.BlockSpec(memory_space=pltpu.MemorySpace.HBM)
        return pl.pallas_call(
            functools.partial(_kernel, M=M, c=c),
            out_shape=jax.ShapeDtypeStruct((1, S, D), bf16),
            in_specs=[any_spec] * 7,
            out_specs=any_spec,
            scratch_shapes=[
                V((S, D), bf16), V((3, D, D), bf16), V((12, D // 2, 128), u32),
                V((D, D), bf16), V((4, 32 * HS, 128), f32), V((4, D // 2, 128), u32),
                V((D,), bf16), V((F, D), bf16), V((F, D), bf16), V((F, D), bf16),
                V((M // 2, D), u32), V((M // 2, D), u32),
                V((4, M, 128), f32), V((4, M, 128), f32),
                V((4, M + PAD, 128), f32), V((4, M + PAD, 128), f32),
                V((4, M + PAD, 128), f32), V((4, M + PAD, 128), f32),
                V((M // 2, D), u32), V((M // 2, D), u32),
                V((4, S, 128), f32), V((S, 128), f32), V((S, 128), f32), V((NB, 8, 128), f32), V((32, D), bf16),
                V((20, D // 2, 128), u32), V((NW, M, 128), f32),
                pltpu.SemaphoreType.DMA((NB,)), pltpu.SemaphoreType.DMA((8,)), pltpu.SemaphoreType.DMA((NB,)),
                pltpu.SemaphoreType.DMA((4,)),
            ],
            compiler_params=pltpu.CompilerParams(vmem_limit_bytes=100 * 1024 * 1024, flags=flags),
        )(A_x, A_wqkv, A_wo, B_w_r, B_w_gate.T, B_w_up.T, B_w_down)
    return fn


_fn = build()


@jax.jit
def pallas_interleave_layers__sliding_local_dilated__moe_arch_mod__prompt_kernel(
    A_x, A_wqkv, A_wo, B_x, B_w_r, B_w_gate, B_w_up, B_w_down
):
    return _fn(A_x, A_wqkv, A_wo, B_x, B_w_r, B_w_gate, B_w_up, B_w_down)
```

```python
import functools

import jax
import jax.numpy as jnp
from jax import lax
import jax.experimental.pallas as pl
import jax.experimental.pallas.tpu as pltpu

S, D, F = 2048, 512, 1376
NW, DIL = 8, 2
EPS = 1e-5
LOG2E = 1.4426950408889634
QSCALE = 0.25 * LOG2E
NEG = -1e9 * LOG2E

M = 512
H = M // 2
NB = S // M
PAD = 16
RC = 16
RA = 8
NCH = M // RC
HS = 17
PR = 64
NP = D // 2 // PR
NT = F // 128
LAST_PARTS = (256, 192, 64)

f32, bf16, u32, i32 = jnp.float32, jnp.bfloat16, jnp.uint32, jnp.int32


def _lane_iota(rows):
    return lax.broadcasted_iota(i32, (rows, 128), 1)


def _row_iota(rows):
    return lax.broadcasted_iota(i32, (rows, 128), 0)


def _cols(i):
    return pl.ds(i * 128, 128)


def _tiles(x):
    return [x[:, i * 128:(i + 1) * 128] for i in range(4)]


def _sum4(a):
    return (a[0] + a[1]) + (a[2] + a[3])


def _chain(a):
    return functools.reduce(lambda x, y: x + y, a)


def _rowsum(x):
    return jnp.broadcast_to(jnp.sum(x, axis=1, keepdims=True), x.shape)


def _row_mean(xs):
    return _rowsum(_sum4(xs)) * (1.0 / D)


def _inv_std(xc):
    return lax.rsqrt(_rowsum(_sum4([x * x for x in xc])) * (1.0 / D) + EPS)


def _pack(x):
    return pltpu.bitcast(x.astype(bf16), u32)


def _mm(a, b):
    return jnp.dot(a, b, preferred_element_type=f32)


class _Plan:
    def __init__(self):
        self.items = []

    def at(self, t, f, *args):
        self.items.append((t, len(self.items), functools.partial(f, *args)))

    def staged(self, span, n, lag, stages, k0=0):
        dt = (span[1] - span[0]) / (n + lag * (len(stages) - 1))
        for k in range(n):
            for s, f in enumerate(stages):
                self.at(span[0] + (k + s * lag) * dt + 1e-6, f, k0 + k)

    def run(self):
        for _, _, f in sorted(self.items, key=lambda e: e[:2]):
            f()


def _kernel(x_hbm, wqkv_hbm, wo_hbm, wr_hbm, wg_hbm, wu_hbm, wd_hbm, out_hbm,
            xb, wraw, wp, woraw, wof, wop, wr_v, wg_v, wu_v, wd_v,
            hb0, hb1, qb0, qb1, kb0, kb1, vb0, vb1, ob0, ob1, x1b, mb, ib, rb, fix, wt,
            sem_x, sem_w, sem_o, sem_q):
    hb, qb, kb, vb, ob = (hb0, hb1), (qb0, qb1), (kb0, kb1), (vb0, vb1), (ob0, ob1)
    live = {}

    def rows(b, off=0, n=M):
        if isinstance(b, int):
            return pl.ds(b * M + off, n)
        return pl.ds(pl.multiple_of(b * M + off, RC), n)

    def x_copy(h0, h1):
        r = pl.ds(h0 * H, (h1 - h0) * H)
        return pltpu.make_async_copy(x_hbm.at[0, r], xb.at[r], sem_x.at[h0])

    def o_copy(b, off=0, nr=M, k=0):
        r = rows(b, off, nr)
        return pltpu.make_async_copy(xb.at[r], out_hbm.at[0, r], sem_o.at[b + k])

    def last_copies():
        return [o_copy(NB - 1, sum(LAST_PARTS[:k]), nr, k) for k, nr in enumerate(LAST_PARTS)]

    def wq_copy(k):
        r = pl.ds(k * D // 2, D // 2)
        return pltpu.make_async_copy(wqkv_hbm.at[r, pl.ds(0, D)], wraw.at[0, r], sem_q.at[k])

    def w_copy(j):
        return pltpu.make_async_copy(wqkv_hbm.at[:, pl.ds(j * D, D)], wraw.at[j], sem_w.at[j])

    def wo_copy():
        return pltpu.make_async_copy(wo_hbm, woraw, sem_w.at[3])

    def wr_copy():
        return pltpu.make_async_copy(wr_hbm, wr_v, sem_w.at[4])

    def ffn_copy(k):
        src, dst = ((wg_hbm, wg_v), (wu_hbm, wu_v), (wd_hbm, wd_v))[k]
        return pltpu.make_async_copy(src, dst, sem_w.at[5 + k])

    def permute_w(j, k):
        r = k * PR
        lane = _lane_iota(PR)
        c0 = ((lane >> 2) & 1) == 1
        c1 = ((lane >> 3) & 1) == 1
        a = [pltpu.bitcast(wraw[j, pl.ds(2 * r, 2 * PR), _cols(i)], u32) for i in range(4)]
        b = [jnp.where(c0, a[i ^ 1], a[i]) for i in range(4)]
        m = [jnp.where(c1, b[i ^ 2], b[i]) for i in range(4)]
        for t in range(4):
            idx = (lane & 7) * 16 + (((lane >> 3) & 3) ^ t) * 4 + (lane >> 5)
            wp[j * 4 + t, pl.ds(r, PR), :] = jnp.take_along_axis(m[t], idx, axis=1)

    def widen_wo(n):
        for h in range(32):
            i = h >> 3
            w = woraw[pl.ds(h * 16, 16), _cols(n)].astype(f32)
            for half in range(2):
                part = w[8 * half:8 * half + 8]
                if i & 1:
                    part = pltpu.roll(part, 4, 0)
                wof[n, pl.ds(h * HS + 8 * (half ^ (i >> 1)), 8), :] = part

    def permute_wo(n):
        for e in range(16):
            for m in range(2):
                lo = wof[n, pl.ds(16 * m * HS + e, 8, stride=2 * HS), :]
                hi = wof[n, pl.ds((16 * m + 1) * HS + e, 8, stride=2 * HS), :]
                wop[n, pl.ds(e * 16 + m * 8, 8), :] = (pltpu.bitcast(lo, u32) >> 16) | pltpu.bitcast(hi, u32)

    def flip(i):
        for k, w in enumerate((wg_v, wu_v)):
            for t in range(4):
                wt[2 * i + k, pl.ds(64 * t, 64), :] = pltpu.bitcast(w[pl.ds(128 * i, 128), _cols(t)].T, u32)

    def ldx(sl):
        return _tiles(xb[sl, :].astype(f32))

    def norm_in1(b, p, k):
        live["in", k] = _row_mean(ldx(rows(b, k * RC, RC)))

    def norm_in2(b, p, k):
        m = live.pop(("in", k))
        xc = [x - m for x in ldx(rows(b, k * RC, RC))]
        inv = _inv_std(xc)
        hb[p][pl.ds(k * 8, 8), :] = _pack(jnp.concatenate([x * inv for x in xc], axis=1))

    def put_qkv(y, p, n, r, nr):
        t = n % 4
        if n < 4:
            qb[p][t, pl.ds(r, nr), :] = y * QSCALE
        else:
            (kb if n < 8 else vb)[p][t, pl.ds(r + PAD, nr), :] = y

    def qkv(p, n, r=0, nr=M):
        h = pltpu.bitcast(hb[p][pl.ds(r // 2, nr // 2), :], bf16)
        put_qkv(_mm(h, pltpu.bitcast(wp[n], bf16)), p, n, r, nr)

    def halo(b, p, do_k=True, do_v=True):
        static = isinstance(b, int)
        for t in range(4):
            if do_k:
                if static and b == 0:
                    kb[p][t, pl.ds(0, PAD), :] = jnp.zeros((PAD, 128), f32)
                else:
                    kb[p][t, pl.ds(0, PAD), :] = kb[1 - p][t, pl.ds(M, PAD), :]
            if do_v:
                if static and b > 0:
                    val = vb[1 - p][t, pl.ds(M, PAD), :]
                else:
                    val = jnp.broadcast_to(vb[p][t, pl.ds(PAD, 1), :], (PAD, 128))
                    if not static:
                        val = jnp.where(b == 0, val, vb[1 - p][t, pl.ds(M, PAD), :])
                vb[p][t, pl.ds(0, PAD), :] = val

    def attn1(p, r, key, nr):
        q = qb[p][:, pl.ds(r, nr), :]
        out = []
        for w in range(NW):
            prod = q * kb[p][:, pl.ds(r + (PAD - DIL * w), nr), :]
            a = _chain([prod[t] for t in range(4)])
            out.append(a + pltpu.roll(a, 64, 1))
        live["qk", key] = out

    def attn2(p, r, key, nr, pos0, dst):
        ls = []
        for w, a in enumerate(live.pop(("qk", key))):
            a = a + pltpu.roll(a, 32, 1)
            if w > 0 and pos0 is not None:
                a = jnp.where(_row_iota(nr) + pos0 >= DIL * w, a, NEG)
            ls.append(a)
        mx = jnp.maximum(jnp.maximum(jnp.maximum(ls[0], ls[1]), jnp.maximum(ls[2], ls[3])),
                         jnp.maximum(jnp.maximum(ls[4], ls[5]), jnp.maximum(ls[6], ls[7])))
        es = [jnp.exp2(a - mx) for a in ls]
        den = _sum4(es[:4]) + _sum4(es[4:])
        y0 = pltpu.reciprocal(den, approx=True)
        inv = y0 * (2.0 - den * y0)
        acc = _chain([es[w][None] * vb[p][:, pl.ds(r + (PAD - DIL * w), nr), :] for w in range(NW)]) * inv[None]
        res = [acc[t] for t in range(4)]
        if nr == 8:
            if key % 2 == 0:
                live["o"] = res
                return
            res = [jnp.concatenate([a, b], axis=0) for a, b in zip(live.pop("o"), res)]
            r = r - 8
        r2 = r // 2 if isinstance(r, int) else pl.multiple_of(r >> 1, 8)
        dst[pl.ds(r2, 8), :] = _pack(jnp.concatenate(res, axis=1))

    def proj(b, src, n, off=0, nr=M):
        o = pltpu.bitcast(src[pl.ds(off // 2, nr // 2), :], bf16)
        y = _mm(o, pltpu.bitcast(wop[n], bf16))
        x1b[n, rows(b, off, nr), :] = y + xb[rows(b, off, nr), _cols(n)].astype(f32)

    def ld1(sl):
        x = x1b[:, sl, :]
        return [x[i] for i in range(4)]

    def load_wr():
        w = wr_v[...].astype(f32).reshape(1, D)
        live["wr"] = [jnp.broadcast_to(w[:, i * 128:(i + 1) * 128], (RC, 128)) for i in range(4)]

    def norm_out1(b, tag, k):
        live["out", tag, k] = _row_mean(ld1(rows(b, k * RC, RC)))

    def norm_out2(b, tag, k, split=False):
        sl = rows(b, k * RC, RC)
        m = live.pop(("out", tag, k))
        xs = ld1(sl)
        xc = [x - m for x in xs]
        var = _rowsum(_sum4([x * x for x in xc]))
        dot = _rowsum(_sum4([xc[i] * live["wr"][i] for i in range(4)]))
        mb[sl, :] = m
        if split:
            live["out", tag, k] = (m, var, dot)
            return
        inv = lax.rsqrt(var * (1.0 / D) + EPS)
        norm_out_store(b, tag, k, [xs[i] + xc[i] * inv for i in range(4)], inv, dot)

    def norm_out3(b, tag, k):
        m, var, dot = live.pop(("out", tag, k))
        inv = lax.rsqrt(var * (1.0 / D) + EPS)
        gain, off = inv + 1.0, m * inv
        norm_out_store(b, tag, k, [x * gain - off for x in ld1(rows(b, k * RC, RC))], inv, dot)

    def norm_out_store(b, tag, k, ys, inv, dot):
        sl = rows(b, k * RC, RC)
        ib[sl, :] = inv
        xb[sl, :] = jnp.concatenate(ys, axis=1).astype(bf16)
        sc = dot * inv
        lane = _lane_iota(8)
        pair = jnp.where((lane & 1) == 1, sc[8:], sc[:8])
        if k == 0:
            live["score", tag] = pair
        else:
            live["score", tag] = jnp.where(((lane >> 1) & (NCH - 1)) == k, pair, live["score", tag])
        if k == NCH - 1:
            rb[b] = live.pop(("score", tag))

    def plan_norm_in(pn, span, b, p, lag, k0=0, n=NCH):
        pn.staged(span, n, lag, [functools.partial(f, b, p) for f in (norm_in1, norm_in2)], k0)

    def plan_norm_out(pn, span, b, tag, lag, three=False, k0=0, n=NCH):
        fs = (norm_out1, functools.partial(norm_out2, split=True), norm_out3) if three else (norm_out1, norm_out2)
        pn.staged(span, n, lag, [functools.partial(f, b, tag) for f in fs], k0)

    def plan_attn(pn, span, b, p, lag, dst, k0=0, n=M // RA):
        def second(k):
            masked = k * RA < DIL * (NW - 1) and not (isinstance(b, int) and b > 0)
            attn2(p, k * RA, k, RA, b * M + k * RA if masked else None, dst)
        pn.staged(span, n, lag, [lambda k: attn1(p, k * RA, k, RA), second], k0)

    def step(j, p):
        def blk(o):
            return (j + o) & (NB - 1)
        for k, at_step in enumerate((3, 4, 4)):
            if at_step % 2 == p:
                pl.when(j == at_step)(lambda k=k: ffn_copy(k).start())
        load_wr()
        pn = _Plan()
        for n in range(4):
            pn.at((n - 0.5) / 16, proj, blk(-2), ob[p], n)
        for n in range(12):
            pn.at((3.5 + n) / 16, qkv, p, n)
        pn.at(2.0, halo, blk(0), p)
        plan_attn(pn, (0, 1.01), blk(-1), 1 - p, 2, ob[1 - p])
        plan_norm_in(pn, (0, 0.55), blk(1), 1 - p, 1.2)
        plan_norm_out(pn, (0.56, 0.96), blk(-2), p, 1)
        pn.run()

    def last_qkv():
        o_copy(NB - 4).start()
        pn = _Plan()
        for n in range(12):
            pn.at(n / 12, qkv, 1, n)
        pn.at(0, halo, NB - 1, 1, True, False)
        pn.at(2.0, halo, NB - 1, 1, False, True)
        plan_attn(pn, (0, 0.7), NB - 2, 0, 1.3, ob[0])
        for i in range(NT // 2):
            pn.at(0.7 + 0.01 * i, flip, NT // 2 - 1 - i)
        pn.run()

    def drain():
        load_wr()
        pn = _Plan()
        for n in range(4):
            pn.at(n * M, proj, NB - 3, ob[1], n)
            pn.at((4 + n) * M, proj, NB - 2, ob[0], n)
        plan_attn(pn, (0, 3329.0), NB - 1, 1, 3.5, hb[0])
        plan_norm_out(pn, (2312.0, 4342.0), NB - 3, 0, 3, True)
        plan_norm_out(pn, (4166.0, 5551.0), NB - 2, 1, 4, True)
        pn.at(4342.0, lambda: o_copy(NB - 3).start())
        pn.at(5551.0, lambda: o_copy(NB - 2).start())
        off = 0
        spans = ((5551.0, 5820.0), (5920.0, 6190.0), (6200.0, 6400.0))
        for nr, span, cp in zip(LAST_PARTS, spans, last_copies()):
            pn.at(span[1], cp.start)
            for n in range(4):
                pn.at(8 * M + 4 * off + n * nr, proj, NB - 1, hb[0], n, off, nr)
            plan_norm_out(pn, span, NB - 1, 2, 4, True, off // RC, nr // RC)
            off += nr
        pn.run()

    def route_ffn(nt, todo):
        last = 128 * NT
        cut = last - 128 * nt
        for i in todo:
            flip(i)

        upper = _lane_iota(8) >= 64
        sc = jnp.concatenate([jnp.where(upper, rb[2 * a + 1], rb[2 * a]) for a in range(NB // 2)], axis=0)
        row = _row_iota(16)
        pos = (row >> 3) * 1024 + _lane_iota(16) * 8 + (row & 7)
        bits = pltpu.bitcast(jnp.where(sc == 0.0, 0.0, sc), i32)
        mono = bits ^ ((bits >> 31) & 0x7FFFFFFF)
        mono = jnp.where(sc == sc, mono, -0x80000000)
        key = pltpu.bitcast((((mono >> 2) + 0x20800000) & ~(S - 1)) | (S - 1 - pos), f32)

        def top(k):
            return jnp.max(jnp.max(k, axis=0, keepdims=True), axis=1, keepdims=True)
        k1 = top(key)
        k2 = top(jnp.where(key == k1, 0.0, key))
        idx = [(S - 1) - (pltpu.bitcast(k, i32)[0, 0] & (S - 1)) for k in (k1, k2)]
        first = row < 8

        def pick(ref, *lead):
            a, b = [jnp.broadcast_to(ref[(*lead, pl.ds(i, 1), slice(None))], (16, 128)) for i in idx]
            return jnp.where(first, a, b)
        m, inv = pick(mb), pick(ib)
        hs = [(pick(x1b, i) - m) * inv for i in range(4)]
        hsel = jnp.concatenate(hs, axis=1).astype(bf16)

        def mm_t(w, r0, nr):
            return lax.dot_general(hsel, w[pl.ds(r0, nr), :], (((1,), (1,)), ((), ())), preferred_element_type=f32)

        def act(g, u):
            return (g * jax.nn.sigmoid(g) * u).astype(bf16)
        g1, u1 = [mm_t(w, last, F - last) for w in (wg_v, wu_v)]
        acts = [act(mm_t(wg_v, 0, cut), mm_t(wu_v, 0, cut))] if cut else []
        for i in range(cut // 128, last // 128):
            acts.append(act(*[_mm(hsel, pltpu.bitcast(wt[2 * i + k], bf16)) for k in range(2)]))
        y = _mm(act(g1, u1), wd_v[pl.ds(last, F - last), :])
        y = y + _mm(jnp.concatenate(acts, axis=1), wd_v[pl.ds(0, last), :])
        load_wr()
        gate = jax.nn.sigmoid(_rowsum(_sum4([hs[i] * live["wr"][i] for i in range(4)])))
        upd = [y[:, i * 128:(i + 1) * 128] * gate for i in range(4)]

        bases = [pl.multiple_of(i & ~15, 16) for i in idx]
        for k in range(2):
            sl = pl.ds(bases[k], 16)
            xs, m, inv = ld1(sl), mb[sl, :], ib[sl, :]
            hit0 = row + bases[k] == idx[0]
            hit1 = row + bases[k] == idx[1]
            for i in range(4):
                a0 = jnp.concatenate([upd[i][:8]] * 2, axis=0)
                a1 = jnp.concatenate([upd[i][8:]] * 2, axis=0)
                add = jnp.where(hit0, a0, jnp.where(hit1, a1, 0.0))
                fix[pl.ds(16 * k, 16), _cols(i)] = (xs[i] + ((xs[i] - m) * inv + add)).astype(bf16)
        return bases

    def mid_fixup(bases):
        for k in range(2):
            xb[pl.ds(bases[k], 16), :] = fix[pl.ds(16 * k, 16), :]
        lo = jnp.minimum(bases[0], bases[1])
        loc = [pl.multiple_of(b & (M - 1), 16) for b in bases]

        @pl.when(lo < 3 * M)
        def _():
            xs = _tiles(fix[...].astype(f32))
            m = _row_mean(xs)
            xc = [x - m for x in xs]
            inv = _inv_std(xc)
            h = jnp.concatenate([x * inv for x in xc], axis=1).astype(bf16)
            for k in range(2):
                @pl.when((bases[k] >= 2 * M) & (bases[k] < 3 * M))
                def _():
                    hb[0][pl.ds(pl.multiple_of(loc[k] >> 1, 8), 8), :] = pltpu.bitcast(h[16 * k:16 * k + 16], u32)

            @pl.when(lo < 2 * M)
            def _():
                ys = [_mm(h, pltpu.bitcast(wp[n], bf16)) for n in range(12)]
                for k in range(2):
                    for p in range(2):
                        @pl.when((bases[k] >= p * M) & (bases[k] < (p + 1) * M))
                        def _():
                            for n in range(12):
                                put_qkv(ys[n][16 * k:16 * k + 16], p, n, loc[k], 16)

            @pl.when(lo < M)
            def _():
                halo(0, 0)
                halo(1, 1)
                rs = loc + [pl.multiple_of(jnp.minimum(r + 16, M - 16), 16) for r in loc]
                for q in range(4):
                    attn1(0, rs[q], q, 16)
                for q in range(4):
                    attn2(0, rs[q], q, 16, rs[q], ob[0])

    def final_fixup(bases):
        for cp in [o_copy(b) for b in range(1, NB - 1)] + last_copies():
            cp.wait()

        def fix_copy(k):
            return pltpu.make_async_copy(fix.at[pl.ds(16 * k, 16)], out_hbm.at[0, pl.ds(bases[k], 16)], sem_o.at[k])
        fix_copy(0).start()

        @pl.when(bases[0] != bases[1])
        def _():
            fix_copy(1).start()
            fix_copy(1).wait()
        fix_copy(0).wait()

    x_copy(0, 1).start()
    for k in range(2):
        wq_copy(k).start()
    x_copy(1, 2).start()
    x_copy(0, 1).wait()
    pn = _Plan()
    plan_norm_in(pn, (0, 1), 0, 0, 3, 0, NCH // 2)
    pn.run()

    w_copy(1).start()
    for k in range(NP):
        if k % (NP // 2) == 0:
            wq_copy(k // (NP // 2)).wait()
        permute_w(0, k)

    x_copy(2, 3).start()
    w_copy(2).start()
    x_copy(1, 2).wait()
    pn = _Plan()
    for n in range(4):
        pn.at(n / 4, qkv, 0, n, 0, H)
    plan_norm_in(pn, (0, 0.8), 0, 0, 2, NCH // 2, NCH // 2)
    pn.run()

    x_copy(3, 4).start()
    wo_copy().start()
    wr_copy().start()
    w_copy(1).wait()
    pn = _Plan()
    for n in range(2):
        pn.at(n, qkv, 0, n, H, H)
    for n in range(4):
        pn.at(2 + n, qkv, 0, 4 + n, 0, H)
    for k in range(NP):
        pn.at(1.5 * k / NP, permute_w, 1, k)
    pn.at(9, halo, 0, 0, True, False)
    pn.run()

    x_copy(4, 6).start()
    x_copy(2, 3).wait()
    w_copy(2).wait()
    pn = _Plan()
    for k in range(NP):
        pn.at(1.5 * k / NP, permute_w, 2, k)
    for n in range(2):
        pn.at(n, qkv, 0, 2 + n, H, H)
    for n in range(4):
        pn.at(2 + n, qkv, 0, 8 + n, 0, H)
    pn.at(7, halo, 0, 0, False, True)
    plan_norm_in(pn, (0.84, 5.77), 1, 1, 1, 0, NCH // 2)
    pn.run()

    x_copy(6, 8).start()
    x_copy(3, 4).wait()
    pn = _Plan()
    for n in range(8):
        pn.at(n, qkv, 0, 4 + n, H, H)
    plan_norm_in(pn, (0, 7), 1, 1, 1, NCH // 2, NCH // 2)
    plan_attn(pn, (0, 8), 0, 0, 2, ob[0], 0, 16)
    pn.run()

    wo_copy().wait()
    wr_copy().wait()
    x_copy(4, 6).wait()
    pn = _Plan()
    for n in range(12):
        pn.at(n / 12, qkv, 1, n)
    for n in range(4):
        pn.at(0.11 + n * 0.13, widen_wo, n)
        pn.at(0.11 + (n + 1.5) * 0.13, permute_wo, n)
    pn.at(2, halo, 1, 1)
    plan_norm_in(pn, (0.18, 0.73), 2, 0, 1)
    plan_attn(pn, (0.02, 0.9), 0, 0, 2, ob[0], 16, M // RA - 16)
    pn.run()
    x_copy(6, 8).wait()

    def layer(l, carry):
        def body(j, carry):
            for p in range(2):
                pl.when((j & 1) == p)(functools.partial(step, j, p))
            return carry
        lax.fori_loop(2 + l * NB, NB + 2 + l * (NB - 3), body, 0)
        pl.when(l == 1)(last_qkv)

        @pl.when(l > 0)
        def _():
            drain()
            o_copy(0).wait()
            final_fixup(route_ffn(NT, ()))

        @pl.when(l == 0)
        def _():
            for k in range(3):
                ffn_copy(k).wait()
            mid_fixup(route_ffn(NT - NT // 2, range(NT // 2, NT)))
        return carry
    lax.fori_loop(0, 2, layer, 0)


@jax.jit
def pallas_interleave_layers__sliding_local_dilated__moe_arch_mod__prompt_kernel(
    A_x: jax.Array,
    A_wqkv: jax.Array,
    A_wo: jax.Array,
    B_x: jax.Array,
    B_w_r: jax.Array,
    B_w_gate: jax.Array,
    B_w_up: jax.Array,
    B_w_down: jax.Array,
):
    del B_x
    vmem = pltpu.VMEM
    hbm = pl.BlockSpec(memory_space=pltpu.MemorySpace.HBM)
    return pl.pallas_call(
        _kernel,
        out_shape=jax.ShapeDtypeStruct((1, S, D), bf16),
        in_specs=[hbm] * 7,
        out_specs=hbm,
        scratch_shapes=[
            vmem((S, D), bf16),
            vmem((3, D, D), bf16), vmem((12, D // 2, 128), u32),
            vmem((D, D), bf16), vmem((4, 40 * HS, 128), f32), vmem((4, D // 2, 128), u32),
            vmem((D,), bf16), vmem((F, D), bf16), vmem((F, D), bf16), vmem((F, D), bf16),
            vmem((M // 2, D), u32), vmem((M // 2, D), u32),
            vmem((4, M, 128), f32), vmem((4, M, 128), f32),
            vmem((4, M + PAD, 128), f32), vmem((4, M + PAD, 128), f32),
            vmem((4, M + PAD, 128), f32), vmem((4, M + PAD, 128), f32),
            vmem((M // 2, D), u32), vmem((M // 2, D), u32),
            vmem((4, S, 128), f32), vmem((S, 128), f32), vmem((S, 128), f32),
            vmem((NB, 8, 128), f32), vmem((32, D), bf16), vmem((2 * NT, D // 2, 128), u32),
            pltpu.SemaphoreType.DMA((8,)), pltpu.SemaphoreType.DMA((8,)),
            pltpu.SemaphoreType.DMA((8,)), pltpu.SemaphoreType.DMA((2,)),
        ],
        compiler_params=pltpu.CompilerParams(vmem_limit_bytes=100 * 1024 * 1024),
    )(A_x, A_wqkv, A_wo, B_w_r, B_w_gate.T, B_w_up.T, B_w_down)
```
